```python
import jax
import jax.numpy as jnp

def _softmax(x, axis=-1):
    return jax.nn.softmax(x, axis=axis)
def _gelu(x):
    return jax.nn.gelu(x, approximate=True)
def _silu(x):
    return jax.nn.silu(x)
def _sigmoid(x):
    return jax.nn.sigmoid(x)
def _layernorm(x, axis=-1, eps=1e-5):
    m = jnp.mean(x, axis=axis, keepdims=True)
    v = jnp.var(x, axis=axis, keepdims=True)
    return (x - m) / jnp.sqrt(v + eps)
def _scatter_add(tgt, idx, src, axis=0):
    return tgt.at[idx].add(src)
def _segment_sum(src, seg, n):
    return jax.ops.segment_sum(src, seg, n)
class _Rng:
    def __init__(self, key):
        self._k = key
    def _next(self):
        self._k, sub = jax.random.split(self._k)
        return sub
    def normal(self, shape):
        return jax.random.normal(self._next(), shape, dtype=jnp.bfloat16)
    def randint(self, lo, hi, shape):
        return jax.random.randint(self._next(), shape, lo, hi, dtype=jnp.int32)
    def uniform(self, shape, lo=0.0, hi=1.0):
        return jax.random.uniform(self._next(), shape, jnp.bfloat16, lo, hi)
    def permutation(self, n):
        return jax.random.permutation(self._next(), n)


kernel_name = 'sequential_preLN__softmax_full_mha__glu_gated_geglu__prompt'

def _fwd_setup_inputs():
    _rng = _Rng(jax.random.key(int.from_bytes(__import__("os").urandom(4), "little")))
    _w = (lambda a: (lambda t: t.astype(jnp.bfloat16) if jnp.issubdtype(t.dtype, jnp.floating) else t)(jnp.asarray(a)))
    def _A_setup():
        B, S, D = 1, 2048, 640
        return {
            "x": _w((lambda *s: _rng.normal(s) * 0.05)(B, S, D)),
            "wqkv": _w((lambda *s: _rng.normal(s) * 0.05)(D, 3 * D)),
            "wo": _w((lambda *s: _rng.normal(s) * 0.05)(D, D)),
        }
    _A_in = _A_setup()

    def _B_setup():
        B, S, Dm, Df = 1, 2048, 640, 1536
        return {
            "x": _w((lambda *s: _rng.normal(s) * 0.05)(B, S, Dm)),
            "w_gate": _w((lambda *s: _rng.normal(s) * 0.05)(Dm, Df) * (Dm ** -0.5)),
            "w_up": _w((lambda *s: _rng.normal(s) * 0.05)(Dm, Df) * (Dm ** -0.5)),
            "w_down": _w((lambda *s: _rng.normal(s) * 0.05)(Df, Dm) * (Df ** -0.5)),
        }
    _B_in = _B_setup()

    return {
        "A_x": _A_in["x"],
        "A_wqkv": _A_in["wqkv"],
        "A_wo": _A_in["wo"],
        "B_x": _B_in["x"],
        "B_w_gate": _B_in["w_gate"],
        "B_w_up": _B_in["w_up"],
        "B_w_down": _B_in["w_down"],
    }

def _fwd_reference(A_x, A_wqkv, A_wo, B_x, B_w_gate, B_w_up, B_w_down):
    def _A_ref(x, wqkv, wo):
        B, S, D = x.shape
        H = 32; Dh = D // H
        qkv = (lambda x, *d: x.transpose(*d))((x @ wqkv).reshape(B, S, 3, H, Dh), 2, 0, 3, 1, 4)
        q, k, v = qkv[0], qkv[1], qkv[2]
        scale = Dh ** -0.5
        scores = jnp.einsum("bhqd,bhkd->bhqk", q, k) * scale
        p = _softmax(scores, axis=-1)
        o = jnp.einsum("bhqk,bhkd->bhqd", p, v)
        return (lambda x, *d: x.transpose(*d))(o, 0, 2, 1, 3).reshape(B, S, D) @ wo

    def _B_ref(x, w_gate, w_up, w_down):
        g = jnp.einsum("bsd,df->bsf", x, w_gate)
        u = jnp.einsum("bsd,df->bsf", x, w_up)
        h = _gelu(g) * u
        return jnp.einsum("bsf,fd->bsd", h, w_down)

    x = A_x
    h = x + _A_ref(_layernorm(x, axis=-1), A_wqkv, A_wo)
    h2 = h + _B_ref(_layernorm(h, axis=-1), B_w_gate, B_w_up, B_w_down)
    return h2


def setup_inputs():
    _inp = _fwd_setup_inputs()
    _gk = jax.random.fold_in(jax.random.key(int.from_bytes(__import__("os").urandom(4), "little")), 2**31 - 1)
    _shapes = [[1, 2048, 640]]
    _dtypes = ['bfloat16']
    _gks = jax.random.split(_gk, len(_shapes))
    _gs = [jax.random.normal(k, s, dtype=jnp.dtype(d)) * 0.05 for k, s, d in zip(_gks, _shapes, _dtypes)]
    _inp["grad_out"] = _gs[0]
    return _inp

def reference(A_x, A_wqkv, A_wo, B_w_gate, B_w_up, B_w_down, B_x, grad_out):
    _const = dict(B_x=B_x)
    def _f(*_d):
        return _fwd_reference(**{'A_x': _d[0], 'A_wqkv': _d[1], 'A_wo': _d[2], 'B_w_gate': _d[3], 'B_w_up': _d[4], 'B_w_down': _d[5], **_const})
    _out, _vjp = jax.vjp(_f, A_x, A_wqkv, A_wo, B_w_gate, B_w_up, B_w_down)
    _grads = _vjp(grad_out)
    _out0 = jnp.asarray(_out)
    return (_out0, *[jnp.asarray(_g) for _g in _grads])
```

```python
import contextlib
import math

import jax
import jax.numpy as jnp
from jax import lax
import jax.experimental.pallas as pl
import jax.experimental.pallas.tpu as pltpu

f32 = jnp.float32
bf16 = jnp.bfloat16
u32 = jnp.uint32

S = 2048
D = 640
DF = 1536
H = 32
DH = 20
HG = 4
HS = 8
NS = H // HS
SR = HS * DH
TQ = 256
NB = S // TQ
NC = 8
NT128 = S // 128
WCH = 128
EPS = 1e-5
SCALE = DH ** -0.5
LOG2E = 1.4426950408889634
LN2 = 0.6931471805599453
QSCALE = SCALE * LOG2E
GELU_C = math.sqrt(2.0 / math.pi)
GELU_A = 0.044715
L_MIN = 2.0 ** -64
FWD_LAG = 5
O_KN, O_VN, O_KT, O_VT, TILE_ROWS = 0, 128, 256, 384, 512
O_P = NT128 * TILE_ROWS
O_QC = O_P + HS * 2 * (S // 2)
O_DO = O_QC + HS * 2 * 16
O_DS = O_DO + HS * 2 * 16
BIG_ROWS = O_DS + 3 * 2 * 128
PROFILE = False

_NT = (((1,), (1,)), ((), ()))


def _scope(name):
    return jax.named_scope(name) if PROFILE else contextlib.nullcontext()


def _dot(a, b):
    return jnp.dot(a, b, preferred_element_type=f32)


def _dot_nt(a, b):
    return lax.dot_general(a, b, _NT, preferred_element_type=f32)


def _pk(v):
    return pltpu.bitcast(v, u32)


def _up(v):
    return pltpu.bitcast(v, bf16)


def _ln_stats(x):
    mu = jnp.mean(x, axis=-1, keepdims=True)
    xc = x - mu
    var = jnp.mean(xc * xc, axis=-1, keepdims=True)
    rstd = lax.rsqrt(var + EPS)
    return xc * rstd, rstd


def _ln_bwd(dy, xhat, rstd):
    m1 = jnp.mean(dy, axis=-1, keepdims=True)
    m2 = jnp.mean(dy * xhat, axis=-1, keepdims=True)
    return rstd * (dy - m1 - xhat * m2)


def _split3(v):
    hi = v.astype(bf16).astype(f32)
    r = v - hi
    mid = r.astype(bf16).astype(f32)
    lo = (r - mid).astype(bf16).astype(f32)
    return hi, mid, lo


def _pad_w(blk, hh):
    jj = hh % HG
    parts = []
    if jj > 0:
        parts.append(jnp.zeros((32 * jj, 128), bf16))
    parts.append(blk)
    if jj < HG - 1:
        parts.append(jnp.zeros((32 * (HG - 1 - jj), 128), bf16))
    return jnp.concatenate(parts, axis=0)


def _kernel(x_hbm, wqkv_hbm, wo_hbm, wg_hbm, wu_hbm, wd_hbm, dy_hbm,
            out_hbm, dx_hbm, dwqkv_hbm, dwo_hbm, dwg_hbm, dwu_hbm, dwd_hbm,
            x_v, dy_v, wqkv_v, wo_v, wg_v, wu_v, wd_v, aT, BIG, QT,
            dQKV, dh_v, dWo, dWg, dWu, dWd, QN, KM, outb,
            ogate, oup, odown, oo,
            x_sems, wq_sems, in_sems, out_sems, w_sems, q_sems, dx_sems):
    row32 = lax.broadcasted_iota(jnp.int32, (32, 128), 0)
    row16 = lax.broadcasted_iota(jnp.int32, (16, 128), 0)

    def x_copy(c):
        rows = pl.ds(pl.multiple_of(c * TQ, TQ), TQ)
        return pltpu.make_async_copy(x_hbm.at[rows, :], x_v.at[rows, :], x_sems.at[c])

    def wq_copy(c):
        rows = pl.ds(pl.multiple_of(c * WCH, WCH), WCH)
        return pltpu.make_async_copy(wqkv_hbm.at[rows, :], wqkv_v.at[rows, :], wq_sems.at[c])

    in_copies = [
        pltpu.make_async_copy(src, dst, in_sems.at[i])
        for i, (src, dst) in enumerate([
            (wd_hbm, wd_v), (dy_hbm, dy_v), (wo_hbm, wo_v), (wg_hbm, wg_v), (wu_hbm, wu_v)])]
    w_copies = [
        pltpu.make_async_copy(src, dst, w_sems.at[i])
        for i, (src, dst) in enumerate([
            (ogate, dwg_hbm), (oup, dwu_hbm), (odown, dwd_hbm), (oo, dwo_hbm)])]

    for c in range(D // WCH):
        wq_copy(c).start()
    x_copy(0).start()
    x_copy(1).start()

    def big(i, off, n):
        return (i, pl.ds(off, n), slice(None))

    def kn(i, hh, t):
        return big(i, t * TILE_ROWS + O_KN + (hh // HG) * 64, 64)

    def vn(i, hh, t):
        return big(i, t * TILE_ROWS + O_VN + (hh // HG) * 64, 64)

    def kt(i, hh, t):
        return big(i, t * TILE_ROWS + O_KT + hh * 16, 16)

    def vt(i, hh, t):
        return big(i, t * TILE_ROWS + O_VT + hh * 16, 16)

    def pp(i, hh, j, t):
        return big(i, O_P + (hh * 2 + j) * (S // 2) + t * 64, 64)

    def qc(i, hh, j):
        return big(i, O_QC + (hh * 2 + j) * 16, 16)

    def do(i, hh, j):
        return big(i, O_DO + (hh * 2 + j) * 16, 16)

    def ds(i, slot, j, kk):
        return big(i, O_DS + slot * 256 + j * 128 + kk * 64, 64)

    def bound_shift(blk, i):
        for j in range(2):
            m = QN[blk * 2 + j, i] * KM[i]
            for hh in range(HS):
                src = QT[blk * 2 + j, i, hh]
                new = jnp.where(row16 == DH - 16, -m[hh:hh + 1], _up(src[8:16]).astype(f32))
                BIG[qc(i, hh, j)] = jnp.concatenate([src[0:8], _pk(new.astype(bf16))], axis=0)

    def prologue(wT, stage, a_s):
        def zero_q(i, carry):
            stage[pl.ds(pl.multiple_of(i * 16, 16), 16), :] = jnp.zeros((16, TQ), f32)
            return carry

        lax.fori_loop(0, D // 16 + 1, zero_q, 0)
        stage[pl.ds(3 * D + 16, 16), :] = jnp.zeros((16, TQ), f32)
        KM[...] = jnp.zeros(KM.shape, f32)

        def tr_w(c, carry):
            c0 = pl.multiple_of(c * WCH, WCH)
            wq_copy(c).wait()
            wT[:, pl.ds(c0, WCH)] = wqkv_v[pl.ds(c0, WCH), :].T
            return carry

        lax.fori_loop(0, D // WCH, tr_w, 0)
        x_copy(0).wait()
        a_s[...] = _ln_stats(x_v[pl.ds(0, TQ), :].astype(f32))[0].astype(bf16)
        for c in range(2, NB):
            x_copy(c).start()

        def extract_q(rc, j):
            t = rc * 2 + j
            lanes = pl.ds(j * 128 if isinstance(j, int) else pl.multiple_of(j * 128, 128), 128)
            for h in range(H):
                q = stage[pl.ds(h * DH, 32), lanes] * QSCALE
                q = jnp.where(row32 < DH, q, 0.0).astype(bf16)
                QT[t, h // HS, h % HS] = _pk(q)
                qf = q.astype(f32)
                QN[t, h // HS, pl.ds(h % HS, 1), :] = jnp.sqrt(
                    jnp.sum(qf * qf, axis=0, keepdims=True))

        def chunk(rc, carry):
            r0 = pl.multiple_of(rc * TQ, TQ)
            rn = jnp.minimum(rc + 1, NB - 1)
            b0 = rc * (2 * TILE_ROWS)

            @pl.when(rc + 1 < NB)
            def _():
                x_copy(rc + 1).wait()

            @pl.when(rc == 1)
            def _():
                for cp in in_copies:
                    cp.start()

            a = a_s[...]
            for j in range(2):
                extract_q(jnp.maximum(rc - 1, 0), j)
            for part in (1, 2, 0):
                prow = pl.ds(part * D + (16 if part else 0), D)
                stage[prow, :] = _dot_nt(wT[pl.ds(part * D, D), :], a)
            aT[:, pl.ds(r0, TQ)] = a.T
            xn = x_v[pl.ds(pl.multiple_of(rn * TQ, TQ), TQ), :]
            a_s[...] = _ln_stats(xn.astype(f32))[0].astype(bf16)
            for part, (offT, offN) in enumerate(((O_KT, O_KN), (O_VT, O_VN))):
                for j in range(2):
                    lanes = pl.ds(j * 128, 128)
                    for g in range(H // HG):
                        blks = []
                        for jj in range(HG):
                            h = g * HG + jj
                            i, hh = h // HS, h % HS
                            v = stage[pl.ds((part + 1) * D + 16 + h * DH, 32), lanes]
                            if part == 0:
                                kb = jnp.where(row32 < DH, v, 0.0).astype(bf16).astype(f32)
                                KM[i, pl.ds(hh, 1), :] = jnp.maximum(
                                    KM[i, pl.ds(hh, 1), :], jnp.sum(kb * kb, axis=0, keepdims=True))
                            v = jnp.where(row32 < DH, v, jnp.where(row32 < DH + 3, 1.0, 0.0)).astype(bf16)
                            off = j * TILE_ROWS + offT + hh * 16
                            BIG[big(i, pl.multiple_of(b0 + off, 16), 16)] = _pk(v)
                            blks.append(v)
                        off = j * TILE_ROWS + offN + (g % 2) * 64
                        BIG[big(g // 2, pl.multiple_of(b0 + off, 64), 64)] = _pk(
                            jnp.concatenate(blks, axis=0).T)
            return carry

        with _scope('proloop'):
            lax.fori_loop(0, NB, chunk, 0)

        def last_q(j, carry):
            extract_q(NB - 1, j)
            return carry

        lax.fori_loop(0, 2, last_q, 0)
        km = jnp.sqrt(jnp.max(KM[...], axis=2, keepdims=True)) * (1.0 + 2.0 ** -6)
        KM[...] = jnp.broadcast_to(km, KM.shape)

    with _scope('prologue'):
        pl.run_scoped(prologue, pltpu.VMEM((3 * D, D), bf16), pltpu.VMEM((3 * D + 32, TQ), f32),
                      pltpu.VMEM((TQ, D), bf16))

    def first_shift(i, carry):
        bound_shift(0, i)
        return carry

    lax.fori_loop(0, NS, first_shift, 0)
    for cp in in_copies:
        cp.wait()

    def out_copy(blk, slot):
        return pltpu.make_async_copy(
            outb.at[slot], out_hbm.at[pl.ds(pl.multiple_of(blk * TQ, TQ), TQ), :], out_sems.at[slot])

    def main(OTn, LI, stage2, bT_s, hhT_s, dg_s, du_s):
        OTn[:, pl.ds(SR, 16), :] = jnp.zeros((NS, 16, TQ), f32)
        stage2[:, pl.ds(SR, 16), :] = jnp.zeros((NS, 16, TQ), f32)
        nsteps = HS * NC

        def fwd_attention(blk):
            def heads(i, carry):
                ot = {}

                def A(t):
                    hh, c = t // NC, t % NC
                    for kk in range(2):
                        for j in range(2):
                            s = _dot(_up(BIG[kn(i, hh, c * 2 + kk)]), _pad_w(_up(BIG[qc(i, hh, j)]), hh))
                            BIG[pp(i, hh, j, c * 2 + kk)] = _pk(jnp.exp2(s).astype(bf16))

                def B(t):
                    hh, c = t // NC, t % NC
                    if c == 0:
                        ot[hh] = [None, None]
                    for kk in range(2):
                        for j in range(2):
                            d = _dot(_up(BIG[vt(i, hh, c * 2 + kk)]), _up(BIG[pp(i, hh, j, c * 2 + kk)]))
                            ot[hh][j] = d if ot[hh][j] is None else ot[hh][j] + d
                    if c == NC - 1:
                        for j in range(2):
                            lanes = pl.ds(j * 128, 128)
                            l = ot[hh][j][DH:DH + 1, :]
                            LI[i, pl.ds(hh, 1), lanes] = l
                            OTn[i, pl.ds(hh * DH, DH), lanes] = ot[hh][j][0:DH, :] * (1.0 / l)

                for t in range(FWD_LAG):
                    A(t)
                for t in range(nsteps):
                    if t + FWD_LAG < nsteps:
                        A(t + FWD_LAG)
                    B(t)
                return carry

            lax.fori_loop(0, NS, heads, 0)

        def exact_max(blk):
            rowblk = lax.broadcasted_iota(jnp.int32, (128, 128), 0) // 32

            def head_tile(n, carry):
                i, hh = n // (2 * HS), (n // 2) % HS
                off = pl.multiple_of(O_QC + (n % (2 * HS)) * 16, 16)
                q = jnp.where(row32 < DH, _up(BIG[big(i, off, 16)]).astype(f32), 0.0)
                w = jnp.where(rowblk == hh % HG, jnp.concatenate([q] * HG, axis=0), 0.0).astype(bf16)

                def tile(it, m):
                    koff = pl.multiple_of(it * TILE_ROWS + O_KN + (hh // HG) * 64, 64)
                    s = _dot(_up(BIG[big(i, koff, 64)]), w)
                    return jnp.maximum(m, jnp.max(s, axis=0, keepdims=True))

                m = lax.fori_loop(0, NT128, tile, jnp.full((1, 128), -jnp.inf, f32))
                hi, mid, lo = _split3(-m)
                q = jnp.where(row32 == DH, hi,
                              jnp.where(row32 == DH + 1, mid, jnp.where(row32 == DH + 2, lo, q)))
                BIG[big(i, off, 16)] = _pk(q.astype(bf16))
                return carry

            lax.fori_loop(0, 2 * H, head_tile, 0)

        def extract_do(i):
            for hh in range(HS):
                for j in range(2):
                    lanes = pl.ds(j * 128, 128)
                    inv = 1.0 / LI[i, pl.ds(hh, 1), lanes]
                    dt = (stage2[i, pl.ds(hh * DH, 32), lanes] * inv).astype(bf16).astype(f32)
                    o = OTn[i, pl.ds(hh * DH, 32), lanes]
                    dd = jnp.sum(jnp.where(row32 < DH, dt * o, 0.0), axis=0, keepdims=True)
                    hi, mid, lo = _split3(-dd)
                    w = jnp.where(row32 < DH, dt,
                                  jnp.where(row32 == DH, hi,
                                            jnp.where(row32 == DH + 1, mid,
                                                      jnp.where(row32 == DH + 2, lo, 0.0))))
                    BIG[do(i, hh, j)] = _pk(w.astype(bf16))

        def bwd_attention(blk):
            def heads(i, carry):
                dq = {}

                def A(t):
                    hh, c = t // NC, t % NC
                    for kk in range(2):
                        for j in range(2):
                            dp = _dot(_up(BIG[vn(i, hh, c * 2 + kk)]), _pad_w(_up(BIG[do(i, hh, j)]), hh))
                            p = _up(BIG[pp(i, hh, j, c * 2 + kk)])
                            BIG[ds(i, t % 3, j, kk)] = _pk((p.astype(f32) * dp).astype(bf16))
                    r = {}
                    for kk in range(2):
                        for j in range(2):
                            r[kk, j] = _dot_nt(_up(BIG[do(i, hh, j)]), _up(BIG[pp(i, hh, j, c * 2 + kk)]))
                    for kk in range(2):
                        idx = (2, c * 2 + kk, i, pl.ds(hh * DH, DH), slice(None))
                        dQKV[idx] = jnp.where(blk == 0, 0.0, dQKV[idx]) + (r[kk, 0] + r[kk, 1])[0:DH]

                def B(t):
                    hh, c = t // NC, t % NC
                    if c == 0:
                        dq[hh] = [None, None]
                    r = {}
                    for kk in range(2):
                        for j in range(2):
                            r[kk, j] = _dot_nt(_up(BIG[qc(i, hh, j)]), _up(BIG[ds(i, t % 3, j, kk)]))
                    for kk in range(2):
                        idx = (1, c * 2 + kk, i, pl.ds(hh * DH, DH), slice(None))
                        dQKV[idx] = (jnp.where(blk == 0, 0.0, dQKV[idx])
                                     + (r[kk, 0] + r[kk, 1])[0:DH] * LN2)
                    for kk in range(2):
                        for j in range(2):
                            d = _dot(_up(BIG[kt(i, hh, c * 2 + kk)]), _up(BIG[ds(i, t % 3, j, kk)]))
                            dq[hh][j] = d if dq[hh][j] is None else dq[hh][j] + d
                    if c == NC - 1:
                        for j in range(2):
                            dQKV[0, blk * 2 + j, i, pl.ds(hh * DH, DH), :] = dq[hh][j][0:DH, :] * SCALE

                def acc_rows(acc_ref, out_ref, rows, new):
                    acc = jnp.where(blk == 0, 0.0, acc_ref[rows, :]) + new
                    acc_ref[rows, :] = acc
                    out_ref[rows, :] = acc.astype(bf16)

                def ffn_wgrads():
                    n1, n2 = D // NS, DF // (2 * NS)
                    bT = _up(bT_s[pl.ds(pl.multiple_of(i * (n1 // 2), 8), n1 // 2), :])
                    rows1 = pl.ds(pl.multiple_of(i * n1, 16), n1)
                    acc_rows(dWg, ogate, rows1, _dot(bT, _up(dg_s[...])))
                    acc_rows(dWu, oup, rows1, _dot(bT, _up(du_s[...])))
                    dy = dy_v[pl.ds(pl.multiple_of(blk * TQ, TQ), TQ), :]
                    for k in range(2):
                        r0 = i * n2 + k * (n2 // 2)
                        hhT = _up(hhT_s[pl.ds(pl.multiple_of(r0, 8), n2 // 2), :])
                        acc_rows(dWd, odown, pl.ds(pl.multiple_of(2 * r0, 16), n2), _dot(hhT, dy))

                A(0)
                A(1)
                for t in range(nsteps):
                    if t + 2 < nsteps:
                        A(t + 2)
                    B(t)
                    if t == nsteps // 2:
                        ffn_wgrads()
                bound_shift((blk + 1) % NB, i)
                return carry

            lax.fori_loop(0, NS, heads, 0)

        def block_body(blk, carry):
            r0 = pl.multiple_of(blk * TQ, TQ)
            rows = pl.ds(r0, TQ)
            slot = blk % 2

            @pl.when(blk >= 2)
            def _():
                out_copy(blk - 2, slot).wait()

            def attempt(state):
                it, _ = state

                @pl.when(it == 1)
                def _():
                    exact_max(blk)

                with _scope('fwd'):
                    fwd_attention(blk)
                lmin = jnp.min(LI[...])
                retry = jnp.logical_and(it == 0, jnp.logical_not(lmin >= L_MIN))
                with _scope('dense'):
                    dense(retry)
                return it + 1, retry

            def dense(retry):
                half = DF // 2
                dy = dy_v[rows, :]
                dhh0 = _dot_nt(dy, wd_v[pl.ds(0, half), :])
                oT = OTn[:, pl.ds(0, SR), :].reshape(D, TQ).astype(bf16)
                hres = x_v[rows, :].astype(f32) + _dot(oT.T, wo_v[...])
                dhh1 = _dot_nt(dy, wd_v[pl.ds(half, half), :])
                bhat, rstd = _ln_stats(hres)
                b = bhat.astype(bf16)
                g_ = _dot(b, wg_v[...])
                u_ = _dot(b, wu_v[...])
                dhh = jnp.concatenate([dhh0, dhh1], axis=1)
                g2 = g_ * g_
                th = jnp.tanh(GELU_C * g_ * (1.0 + GELU_A * g2))
                ge = 0.5 * g_ * (1.0 + th)
                gd = 0.5 * (1.0 + th) + 0.5 * g_ * (1.0 - th * th) * (GELU_C * (1.0 + 3.0 * GELU_A * g2))
                hh = (ge * u_).astype(bf16)
                dg = (dhh * u_ * gd).astype(bf16)
                du = (dhh * ge).astype(bf16)
                db = _dot_nt(dg, wg_v[...]) + _dot_nt(du, wu_v[...])
                outb[slot] = (hres + _dot(hh, wd_v[...])).astype(bf16)
                dh = dy.astype(f32) + _ln_bwd(db, bhat, rstd)
                dh_v[rows, :] = dh
                dhb = dh.astype(bf16)
                stage2[:, pl.ds(0, SR), :] = _dot_nt(wo_v[...], dhb).reshape(NS, SR, TQ)
                bT_s[...] = _pk(b.T)
                hhT_s[...] = _pk(hh.T)
                dg_s[...] = _pk(dg)
                du_s[...] = _pk(du)
                base = jnp.where(blk == 0, 0.0, dWo[...])
                acc = jnp.where(retry, base, base + _dot(oT, dhb))
                dWo[...] = acc
                oo[...] = acc.astype(bf16)
                for i in range(NS):
                    extract_do(i)

            with _scope('while'):
                lax.while_loop(lambda st: st[1], attempt, (jnp.int32(0), True))
            out_copy(blk, slot).start()

            with _scope('bwd'):
                bwd_attention(blk)
            return carry

        with _scope('main'):
            lax.fori_loop(0, NB, block_body, 0)

    pl.run_scoped(
        main,
        pltpu.VMEM((NS, SR + 16, TQ), f32),
        pltpu.VMEM((NS, HS, TQ), f32),
        pltpu.VMEM((NS, SR + 16, TQ), f32),
        pltpu.VMEM((D // 2, TQ), u32),
        pltpu.VMEM((DF // 2, TQ), u32),
        pltpu.VMEM((TQ // 2, DF), u32),
        pltpu.VMEM((TQ // 2, DF), u32),
    )

    for cp in w_copies:
        cp.start()

    def epilogue(oqkv):
        dflat = dQKV.reshape(3, NT128, D, 128)

        def qkv_copy(c):
            cols = pl.ds(pl.multiple_of(c * 128, 128), 128)
            return pltpu.make_async_copy(oqkv.at[:, cols], dwqkv_hbm.at[:, cols], q_sems.at[c])

        def dx_copy(t):
            rows = pl.ds(pl.multiple_of(t * 128, 128), 128)
            return pltpu.make_async_copy(dy_v.at[rows, :], dx_hbm.at[rows, :], dx_sems.at[t])

        def dx_tile(t, between):
            rows = pl.ds(pl.multiple_of(t * 128, 128), 128)
            da = _dot(wqkv_v[...], dQKV[:, t].reshape(3 * D, 128).astype(bf16)).T
            between()
            xhat, rstd = _ln_stats(x_v[rows, :].astype(f32))
            dx = dh_v[rows, :] + _ln_bwd(da, xhat, rstd)
            dy_v[rows, :] = dx.astype(bf16)
            dx_copy(t).start()

        def tail(t, carry):
            def dw():
                c = jnp.minimum(t, 14)
                rows = pl.ds(pl.multiple_of((c % 5) * 128, 128), 128)
                w = jnp.concatenate(
                    [dflat[c // 5, i, rows, :].astype(bf16) for i in range(NT128)], axis=1)
                oqkv[:, pl.ds(pl.multiple_of(t * 128, 128), 128)] = _dot_nt(aT[...], w).astype(bf16)

            @pl.when(t >= 1)
            def _():
                qkv_copy(t - 1).start()

            dx_tile(t, dw)
            return carry

        with _scope('tail'):
            lax.fori_loop(0, NT128, tail, 0)
        out_copy(NB - 2, 0).wait()
        out_copy(NB - 1, 1).wait()
        for cp in w_copies:
            cp.wait()

        def drain(t, carry):
            qkv_copy(t - 1).wait()
            dx_copy(t).wait()
            return carry

        dx_copy(0).wait()
        lax.fori_loop(1, NT128, drain, 0)

    pl.run_scoped(epilogue, pltpu.VMEM((D, S), bf16))


@jax.jit
def pallas_sequential_preLN__softmax_full_mha__glu_gated_geglu__prompt_kernel(
    A_x: jax.Array,
    A_wqkv: jax.Array,
    A_wo: jax.Array,
    B_x: jax.Array,
    B_w_gate: jax.Array,
    B_w_up: jax.Array,
    B_w_down: jax.Array,
    grad_out: jax.Array,
):
    del B_x
    x = A_x.reshape(S, D)
    dy = grad_out.reshape(S, D)
    any_spec = pl.BlockSpec(memory_space=pl.ANY)
    out_shape = (
        jax.ShapeDtypeStruct((S, D), bf16),
        jax.ShapeDtypeStruct((S, D), bf16),
        jax.ShapeDtypeStruct((D, 3 * D), bf16),
        jax.ShapeDtypeStruct((D, D), bf16),
        jax.ShapeDtypeStruct((D, DF), bf16),
        jax.ShapeDtypeStruct((D, DF), bf16),
        jax.ShapeDtypeStruct((DF, D), bf16),
    )
    scratch = [
        pltpu.VMEM((S, D), bf16),
        pltpu.VMEM((S, D), bf16),
        pltpu.VMEM((D, 3 * D), bf16),
        pltpu.VMEM((D, D), bf16),
        pltpu.VMEM((D, DF), bf16),
        pltpu.VMEM((D, DF), bf16),
        pltpu.VMEM((DF, D), bf16),
        pltpu.VMEM((D, S), bf16),
        pltpu.VMEM((NS, BIG_ROWS, 128), u32),
        pltpu.VMEM((NT128, NS, HS, 16, 128), u32),
        pltpu.VMEM((3, NT128, NS, SR, 128), f32),
        pltpu.VMEM((S, D), f32),
        pltpu.VMEM((D, D), f32),
        pltpu.VMEM((D, DF), f32),
        pltpu.VMEM((D, DF), f32),
        pltpu.VMEM((DF, D), f32),
        pltpu.VMEM((NT128, NS, HS, 128), f32),
        pltpu.VMEM((NS, HS, 128), f32),
        pltpu.VMEM((2, TQ, D), bf16),
        pltpu.VMEM((D, DF), bf16),
        pltpu.VMEM((D, DF), bf16),
        pltpu.VMEM((DF, D), bf16),
        pltpu.VMEM((D, D), bf16),
        pltpu.SemaphoreType.DMA((NB,)),
        pltpu.SemaphoreType.DMA((D // WCH,)),
        pltpu.SemaphoreType.DMA((5,)),
        pltpu.SemaphoreType.DMA((2,)),
        pltpu.SemaphoreType.DMA((4,)),
        pltpu.SemaphoreType.DMA((3 * D // 128,)),
        pltpu.SemaphoreType.DMA((NT128,)),
    ]
    out, dx, dwqkv, dwo, dwg, dwu, dwd = pl.pallas_call(
        _kernel,
        out_shape=out_shape,
        in_specs=[any_spec] * 7,
        out_specs=tuple([any_spec] * 7),
        scratch_shapes=scratch,
        compiler_params=pltpu.CompilerParams(vmem_limit_bytes=127 * 1024 * 1024),
    )(x, A_wqkv, A_wo, B_w_gate, B_w_up, B_w_down, dy)
    return (out.reshape(1, S, D), dx.reshape(1, S, D), dwqkv, dwo, dwg, dwu, dwd)
```

```python
import contextlib
import math

import jax
import jax.numpy as jnp
from jax import lax
import jax.experimental.pallas as pl
import jax.experimental.pallas.tpu as pltpu

f32 = jnp.float32
bf16 = jnp.bfloat16
u32 = jnp.uint32

S = 2048
D = 640
DF = 1536
H = 32
DH = 20
HG = 4
HS = 8
NS = H // HS
SR = HS * DH
TQ = 256
NB = S // TQ
NC = 8
NT128 = S // 128
WCH = 128
EPS = 1e-5
SCALE = DH ** -0.5
LOG2E = 1.4426950408889634
LN2 = 0.6931471805599453
QSCALE = SCALE * LOG2E
GELU_C = math.sqrt(2.0 / math.pi)
GELU_A = 0.044715
L_MIN = 2.0 ** -64
FWD_LAG = 6
O_KN, O_VN, O_KT, O_VT, TILE_ROWS = 0, 128, 256, 384, 512
O_P = NT128 * TILE_ROWS
O_QC = O_P + HS * 2 * (S // 2)
O_DO = O_QC + HS * 2 * 16
O_DS = O_DO + HS * 2 * 16
BIG_ROWS = O_DS + 3 * 2 * 128
PROFILE = False

_NT = (((1,), (1,)), ((), ()))


def _scope(name):
    return jax.named_scope(name) if PROFILE else contextlib.nullcontext()


def _dot(a, b):
    return jnp.dot(a, b, preferred_element_type=f32)


def _dot_nt(a, b):
    return lax.dot_general(a, b, _NT, preferred_element_type=f32)


def _pk(v):
    return pltpu.bitcast(v, u32)


def _up(v):
    return pltpu.bitcast(v, bf16)


def _ln_stats(x):
    mu = jnp.mean(x, axis=-1, keepdims=True)
    xc = x - mu
    var = jnp.mean(xc * xc, axis=-1, keepdims=True)
    rstd = lax.rsqrt(var + EPS)
    return xc * rstd, rstd


def _ln_bwd(dy, xhat, rstd):
    m1 = jnp.mean(dy, axis=-1, keepdims=True)
    m2 = jnp.mean(dy * xhat, axis=-1, keepdims=True)
    return rstd * (dy - m1 - xhat * m2)


def _split3(v):
    hi = v.astype(bf16).astype(f32)
    r = v - hi
    mid = r.astype(bf16).astype(f32)
    lo = (r - mid).astype(bf16).astype(f32)
    return hi, mid, lo


def _pad_w(blk, hh):
    jj = hh % HG
    parts = []
    if jj > 0:
        parts.append(jnp.zeros((32 * jj, 128), bf16))
    parts.append(blk)
    if jj < HG - 1:
        parts.append(jnp.zeros((32 * (HG - 1 - jj), 128), bf16))
    return jnp.concatenate(parts, axis=0)


def _kernel(x_hbm, wqkv_hbm, wo_hbm, wg_hbm, wu_hbm, wd_hbm, dy_hbm,
            out_hbm, dx_hbm, dwqkv_hbm, dwo_hbm, dwg_hbm, dwu_hbm, dwd_hbm,
            x_v, dy_v, wqkv_v, wo_v, wg_v, wu_v, wd_v, aT, BIG, QT,
            dQKV, dh_v, dWo, dWg, dWu, dWd, QN, KM, outb,
            ogate, oup, odown, oo,
            x_sems, wq_sems, in_sems, out_sems, w_sems, q_sems, dx_sems):
    row32 = lax.broadcasted_iota(jnp.int32, (32, 128), 0)
    row16 = lax.broadcasted_iota(jnp.int32, (16, 128), 0)

    def x_copy(c):
        rows = pl.ds(pl.multiple_of(c * TQ, TQ), TQ)
        return pltpu.make_async_copy(x_hbm.at[rows, :], x_v.at[rows, :], x_sems.at[c])

    def wq_copy(c):
        rows = pl.ds(pl.multiple_of(c * WCH, WCH), WCH)
        return pltpu.make_async_copy(wqkv_hbm.at[rows, :], wqkv_v.at[rows, :], wq_sems.at[c])

    in_copies = [
        pltpu.make_async_copy(src, dst, in_sems.at[i])
        for i, (src, dst) in enumerate([
            (wd_hbm, wd_v), (dy_hbm, dy_v), (wo_hbm, wo_v), (wg_hbm, wg_v), (wu_hbm, wu_v)])]
    w_copies = [
        pltpu.make_async_copy(src, dst, w_sems.at[i])
        for i, (src, dst) in enumerate([
            (ogate, dwg_hbm), (oup, dwu_hbm), (odown, dwd_hbm), (oo, dwo_hbm)])]

    for c in range(D // WCH):
        wq_copy(c).start()
    x_copy(0).start()
    x_copy(1).start()

    def big(i, off, n):
        return (i, pl.ds(off, n), slice(None))

    def kn(i, hh, t):
        return big(i, t * TILE_ROWS + O_KN + (hh // HG) * 64, 64)

    def vn(i, hh, t):
        return big(i, t * TILE_ROWS + O_VN + (hh // HG) * 64, 64)

    def kt(i, hh, t):
        return big(i, t * TILE_ROWS + O_KT + hh * 16, 16)

    def vt(i, hh, t):
        return big(i, t * TILE_ROWS + O_VT + hh * 16, 16)

    def pp(i, hh, j, t):
        return big(i, O_P + (hh * 2 + j) * (S // 2) + t * 64, 64)

    def qc(i, hh, j):
        return big(i, O_QC + (hh * 2 + j) * 16, 16)

    def do(i, hh, j):
        return big(i, O_DO + (hh * 2 + j) * 16, 16)

    def ds(i, slot, j, kk):
        return big(i, O_DS + slot * 256 + j * 128 + kk * 64, 64)

    def bound_shift(blk, i):
        for j in range(2):
            m = QN[blk * 2 + j, i] * KM[i]
            for hh in range(HS):
                src = QT[blk * 2 + j, i, hh]
                new = jnp.where(row16 == DH - 16, -m[hh:hh + 1], _up(src[8:16]).astype(f32))
                BIG[qc(i, hh, j)] = jnp.concatenate([src[0:8], _pk(new.astype(bf16))], axis=0)

    def prologue(wT, stage, a_s):
        def zero_q(i, carry):
            stage[pl.ds(pl.multiple_of(i * 16, 16), 16), :] = jnp.zeros((16, TQ), f32)
            return carry

        lax.fori_loop(0, D // 16 + 1, zero_q, 0)
        stage[pl.ds(3 * D + 16, 16), :] = jnp.zeros((16, TQ), f32)
        KM[...] = jnp.zeros(KM.shape, f32)

        def tr_w(c, carry):
            c0 = pl.multiple_of(c * WCH, WCH)
            wq_copy(c).wait()
            wT[:, pl.ds(c0, WCH)] = wqkv_v[pl.ds(c0, WCH), :].T
            return carry

        lax.fori_loop(0, D // WCH, tr_w, 0)
        x_copy(0).wait()
        a_s[...] = _ln_stats(x_v[pl.ds(0, TQ), :].astype(f32))[0].astype(bf16)
        for c in range(2, NB):
            x_copy(c).start()

        def extract_q(rc, j):
            t = rc * 2 + j
            lanes = pl.ds(j * 128 if isinstance(j, int) else pl.multiple_of(j * 128, 128), 128)
            for h in range(H):
                q = stage[pl.ds(h * DH, 32), lanes] * QSCALE
                q = jnp.where(row32 < DH, q, 0.0).astype(bf16)
                QT[t, h // HS, h % HS] = _pk(q)
                qf = q.astype(f32)
                QN[t, h // HS, pl.ds(h % HS, 1), :] = jnp.sqrt(
                    jnp.sum(qf * qf, axis=0, keepdims=True))

        def chunk(rc, carry):
            r0 = pl.multiple_of(rc * TQ, TQ)
            rn = jnp.minimum(rc + 1, NB - 1)
            b0 = rc * (2 * TILE_ROWS)

            @pl.when(rc + 1 < NB)
            def _():
                x_copy(rc + 1).wait()

            @pl.when(rc == 1)
            def _():
                for cp in in_copies:
                    cp.start()

            a = a_s[...]
            for j in range(2):
                extract_q(jnp.maximum(rc - 1, 0), j)
            for part in (1, 2, 0):
                prow = pl.ds(part * D + (16 if part else 0), D)
                stage[prow, :] = _dot_nt(wT[pl.ds(part * D, D), :], a)
            aT[:, pl.ds(r0, TQ)] = a.T
            xn = x_v[pl.ds(pl.multiple_of(rn * TQ, TQ), TQ), :]
            a_s[...] = _ln_stats(xn.astype(f32))[0].astype(bf16)
            for part, (offT, offN) in enumerate(((O_KT, O_KN), (O_VT, O_VN))):
                for j in range(2):
                    lanes = pl.ds(j * 128, 128)
                    for g in range(H // HG):
                        blks = []
                        for jj in range(HG):
                            h = g * HG + jj
                            i, hh = h // HS, h % HS
                            v = stage[pl.ds((part + 1) * D + 16 + h * DH, 32), lanes]
                            if part == 0:
                                kb = jnp.where(row32 < DH, v, 0.0).astype(bf16).astype(f32)
                                KM[i, pl.ds(hh, 1), :] = jnp.maximum(
                                    KM[i, pl.ds(hh, 1), :], jnp.sum(kb * kb, axis=0, keepdims=True))
                            v = jnp.where(row32 < DH, v, jnp.where(row32 < DH + 3, 1.0, 0.0)).astype(bf16)
                            off = j * TILE_ROWS + offT + hh * 16
                            BIG[big(i, pl.multiple_of(b0 + off, 16), 16)] = _pk(v)
                            blks.append(v)
                        off = j * TILE_ROWS + offN + (g % 2) * 64
                        BIG[big(g // 2, pl.multiple_of(b0 + off, 64), 64)] = _pk(
                            jnp.concatenate(blks, axis=0).T)
            return carry

        with _scope('proloop'):
            lax.fori_loop(0, NB, chunk, 0)

        def last_q(j, carry):
            extract_q(NB - 1, j)
            return carry

        lax.fori_loop(0, 2, last_q, 0)
        km = jnp.sqrt(jnp.max(KM[...], axis=2, keepdims=True)) * (1.0 + 2.0 ** -6)
        KM[...] = jnp.broadcast_to(km, KM.shape)

    with _scope('prologue'):
        pl.run_scoped(prologue, pltpu.VMEM((3 * D, D), bf16), pltpu.VMEM((3 * D + 32, TQ), f32),
                      pltpu.VMEM((TQ, D), bf16))

    def first_shift(i, carry):
        bound_shift(0, i)
        return carry

    lax.fori_loop(0, NS, first_shift, 0)
    for cp in in_copies:
        cp.wait()

    def out_copy(blk, slot):
        return pltpu.make_async_copy(
            outb.at[slot], out_hbm.at[pl.ds(pl.multiple_of(blk * TQ, TQ), TQ), :], out_sems.at[slot])

    def main(OTn, LI, stage2, bT_s, hhT_s, dg_s, du_s):
        OTn[:, pl.ds(SR, 16), :] = jnp.zeros((NS, 16, TQ), f32)
        stage2[:, pl.ds(SR, 16), :] = jnp.zeros((NS, 16, TQ), f32)
        nsteps = HS * NC

        def fwd_attention(blk):
            def heads(i, carry):
                ot = {}

                def A(t):
                    hh, c = t // NC, t % NC
                    for kk in range(2):
                        for j in range(2):
                            s = _dot(_up(BIG[kn(i, hh, c * 2 + kk)]), _pad_w(_up(BIG[qc(i, hh, j)]), hh))
                            BIG[pp(i, hh, j, c * 2 + kk)] = _pk(jnp.exp2(s).astype(bf16))

                def B(t):
                    hh, c = t // NC, t % NC
                    if c == 0:
                        ot[hh] = [None, None]
                    for kk in range(2):
                        for j in range(2):
                            d = _dot(_up(BIG[vt(i, hh, c * 2 + kk)]), _up(BIG[pp(i, hh, j, c * 2 + kk)]))
                            ot[hh][j] = d if ot[hh][j] is None else ot[hh][j] + d
                    if c == NC - 1:
                        for j in range(2):
                            lanes = pl.ds(j * 128, 128)
                            l = ot[hh][j][DH:DH + 1, :]
                            LI[i, pl.ds(hh, 1), lanes] = l
                            OTn[i, pl.ds(hh * DH, DH), lanes] = ot[hh][j][0:DH, :] * (1.0 / l)

                for t in range(FWD_LAG):
                    A(t)
                for t in range(nsteps):
                    if t + FWD_LAG < nsteps:
                        A(t + FWD_LAG)
                    B(t)
                return carry

            lax.fori_loop(0, NS, heads, 0)

        def exact_max(blk):
            rowblk = lax.broadcasted_iota(jnp.int32, (128, 128), 0) // 32

            def head_tile(n, carry):
                i, hh = n // (2 * HS), (n // 2) % HS
                off = pl.multiple_of(O_QC + (n % (2 * HS)) * 16, 16)
                q = jnp.where(row32 < DH, _up(BIG[big(i, off, 16)]).astype(f32), 0.0)
                w = jnp.where(rowblk == hh % HG, jnp.concatenate([q] * HG, axis=0), 0.0).astype(bf16)

                def tile(it, m):
                    koff = pl.multiple_of(it * TILE_ROWS + O_KN + (hh // HG) * 64, 64)
                    s = _dot(_up(BIG[big(i, koff, 64)]), w)
                    return jnp.maximum(m, jnp.max(s, axis=0, keepdims=True))

                m = lax.fori_loop(0, NT128, tile, jnp.full((1, 128), -jnp.inf, f32))
                hi, mid, lo = _split3(-m)
                q = jnp.where(row32 == DH, hi,
                              jnp.where(row32 == DH + 1, mid, jnp.where(row32 == DH + 2, lo, q)))
                BIG[big(i, off, 16)] = _pk(q.astype(bf16))
                return carry

            lax.fori_loop(0, 2 * H, head_tile, 0)

        def extract_do(i):
            for hh in range(HS):
                for j in range(2):
                    lanes = pl.ds(j * 128, 128)
                    inv = 1.0 / LI[i, pl.ds(hh, 1), lanes]
                    dt = (stage2[i, pl.ds(hh * DH, 32), lanes] * inv).astype(bf16).astype(f32)
                    o = OTn[i, pl.ds(hh * DH, 32), lanes]
                    dd = jnp.sum(jnp.where(row32 < DH, dt * o, 0.0), axis=0, keepdims=True)
                    hi, mid, lo = _split3(-dd)
                    w = jnp.where(row32 < DH, dt,
                                  jnp.where(row32 == DH, hi,
                                            jnp.where(row32 == DH + 1, mid,
                                                      jnp.where(row32 == DH + 2, lo, 0.0))))
                    BIG[do(i, hh, j)] = _pk(w.astype(bf16))

        def bwd_attention(blk):
            def heads(i, carry):
                dq = {}

                def A(t):
                    hh, c = t // NC, t % NC
                    for kk in range(2):
                        for j in range(2):
                            dp = _dot(_up(BIG[vn(i, hh, c * 2 + kk)]), _pad_w(_up(BIG[do(i, hh, j)]), hh))
                            p = _up(BIG[pp(i, hh, j, c * 2 + kk)])
                            BIG[ds(i, t % 3, j, kk)] = _pk((p.astype(f32) * dp).astype(bf16))
                    r = {}
                    for kk in range(2):
                        for j in range(2):
                            r[kk, j] = _dot_nt(_up(BIG[do(i, hh, j)]), _up(BIG[pp(i, hh, j, c * 2 + kk)]))
                    for kk in range(2):
                        idx = (2, c * 2 + kk, i, pl.ds(hh * DH, DH), slice(None))
                        dQKV[idx] = jnp.where(blk == 0, 0.0, dQKV[idx]) + (r[kk, 0] + r[kk, 1])[0:DH]

                def BK(t):
                    hh, c = t // NC, t % NC
                    r = {}
                    for kk in range(2):
                        for j in range(2):
                            r[kk, j] = _dot_nt(_up(BIG[qc(i, hh, j)]), _up(BIG[ds(i, t % 3, j, kk)]))
                    for kk in range(2):
                        idx = (1, c * 2 + kk, i, pl.ds(hh * DH, DH), slice(None))
                        dQKV[idx] = (jnp.where(blk == 0, 0.0, dQKV[idx])
                                     + (r[kk, 0] + r[kk, 1])[0:DH] * LN2)

                def BQ(t):
                    hh, c = t // NC, t % NC
                    if c == 0:
                        dq[hh] = [None, None]
                    for kk in range(2):
                        for j in range(2):
                            d = _dot(_up(BIG[kt(i, hh, c * 2 + kk)]), _up(BIG[ds(i, t % 3, j, kk)]))
                            dq[hh][j] = d if dq[hh][j] is None else dq[hh][j] + d
                    if c == NC - 1:
                        for j in range(2):
                            dQKV[0, blk * 2 + j, i, pl.ds(hh * DH, DH), :] = dq[hh][j][0:DH, :] * SCALE

                def acc_rows(acc_ref, out_ref, rows, cols, new):
                    acc = jnp.where(blk == 0, 0.0, acc_ref[rows, cols]) + new
                    acc_ref[rows, cols] = acc
                    out_ref[rows, cols] = acc.astype(bf16)

                n1, n2 = D // NS, DF // (2 * NS)

                def dwd_piece(k, c0, nc):
                    r0 = i * n2 + k * (n2 // 2)
                    hhT = _up(hhT_s[pl.ds(pl.multiple_of(r0, 8), n2 // 2), :])
                    cols = pl.ds(c0, nc)
                    dy = dy_v[pl.ds(pl.multiple_of(blk * TQ, TQ), TQ), cols]
                    acc_rows(dWd, odown, pl.ds(pl.multiple_of(2 * r0, 16), n2), cols, _dot(hhT, dy))

                def ffn_wgrads():
                    bT = _up(bT_s[pl.ds(pl.multiple_of(i * (n1 // 2), 8), n1 // 2), :])
                    rows1 = pl.ds(pl.multiple_of(i * n1, 16), n1)
                    acc_rows(dWg, ogate, rows1, slice(None), _dot(bT, _up(dg_s[...])))
                    acc_rows(dWu, oup, rows1, slice(None), _dot(bT, _up(du_s[...])))
                    dwd_piece(0, 0, D)
                    dwd_piece(1, 256, D - 256)

                A(0)
                A(1)
                for t in range(nsteps - 2):
                    A(t + 2)
                    BK(t)
                    BQ(t)
                    if t == nsteps // 2:
                        ffn_wgrads()
                dwd_piece(1, 0, 256)
                BK(nsteps - 2)
                BK(nsteps - 1)
                BQ(nsteps - 2)
                BQ(nsteps - 1)
                bound_shift((blk + 1) % NB, i)
                return carry

            lax.fori_loop(0, NS, heads, 0)

        def block_body(blk, carry):
            r0 = pl.multiple_of(blk * TQ, TQ)
            rows = pl.ds(r0, TQ)
            slot = blk % 2

            @pl.when(blk >= 2)
            def _():
                out_copy(blk - 2, slot).wait()

            def attempt(state):
                it, _ = state

                @pl.when(it == 1)
                def _():
                    exact_max(blk)

                with _scope('fwd'):
                    fwd_attention(blk)
                lmin = jnp.min(LI[...])
                retry = jnp.logical_and(it == 0, jnp.logical_not(lmin >= L_MIN))
                with _scope('dense'):
                    dense(retry)
                return it + 1, retry

            def dense(retry):
                half = DF // 2
                dy = dy_v[rows, :]
                dhh0 = _dot_nt(dy, wd_v[pl.ds(0, half), :])
                oT = OTn[:, pl.ds(0, SR), :].reshape(D, TQ).astype(bf16)
                hres = x_v[rows, :].astype(f32) + _dot(oT.T, wo_v[...])
                dhh1 = _dot_nt(dy, wd_v[pl.ds(half, half), :])
                bhat, rstd = _ln_stats(hres)
                b = bhat.astype(bf16)
                g_ = _dot(b, wg_v[...])
                u_ = _dot(b, wu_v[...])
                dhh = jnp.concatenate([dhh0, dhh1], axis=1)
                g2 = g_ * g_
                th = jnp.tanh(GELU_C * g_ * (1.0 + GELU_A * g2))
                ge = 0.5 * g_ * (1.0 + th)
                gd = 0.5 * (1.0 + th) + 0.5 * g_ * (1.0 - th * th) * (GELU_C * (1.0 + 3.0 * GELU_A * g2))
                hh = (ge * u_).astype(bf16)
                dg = (dhh * u_ * gd).astype(bf16)
                du = (dhh * ge).astype(bf16)
                db = _dot_nt(dg, wg_v[...]) + _dot_nt(du, wu_v[...])
                outb[slot] = (hres + _dot(hh, wd_v[...])).astype(bf16)
                dh = dy.astype(f32) + _ln_bwd(db, bhat, rstd)
                dh_v[rows, :] = dh
                dhb = dh.astype(bf16)
                stage2[:, pl.ds(0, SR), :] = _dot_nt(wo_v[...], dhb).reshape(NS, SR, TQ)
                bT_s[...] = _pk(b.T)
                hhT_s[...] = _pk(hh.T)
                dg_s[...] = _pk(dg)
                du_s[...] = _pk(du)
                base = jnp.where(blk == 0, 0.0, dWo[...])
                acc = jnp.where(retry, base, base + _dot(oT, dhb))
                dWo[...] = acc
                oo[...] = acc.astype(bf16)
                for i in range(NS):
                    extract_do(i)

            with _scope('while'):
                lax.while_loop(lambda st: st[1], attempt, (jnp.int32(0), True))
            out_copy(blk, slot).start()

            with _scope('bwd'):
                bwd_attention(blk)
            return carry

        with _scope('main'):
            lax.fori_loop(0, NB, block_body, 0)

    pl.run_scoped(
        main,
        pltpu.VMEM((NS, SR + 16, TQ), f32),
        pltpu.VMEM((NS, HS, TQ), f32),
        pltpu.VMEM((NS, SR + 16, TQ), f32),
        pltpu.VMEM((D // 2, TQ), u32),
        pltpu.VMEM((DF // 2, TQ), u32),
        pltpu.VMEM((TQ // 2, DF), u32),
        pltpu.VMEM((TQ // 2, DF), u32),
    )

    for cp in w_copies:
        cp.start()

    def epilogue(oqkv, last):
        dflat = dQKV.reshape(3, NT128, D, 128)

        def qkv_copy(c):
            cols = pl.ds(pl.multiple_of(c * 128, 128), 128)
            return pltpu.make_async_copy(oqkv.at[:, cols], dwqkv_hbm.at[:, cols], q_sems.at[c])

        def dx_copy(t):
            rows = pl.ds(pl.multiple_of(t * 128, 128), 128)
            return pltpu.make_async_copy(dy_v.at[rows, :], dx_hbm.at[rows, :], dx_sems.at[t])

        def dx_finish(t, daT):
            rows = pl.ds(pl.multiple_of(t * 128, 128), 128)
            xhat, rstd = _ln_stats(x_v[rows, :].astype(f32))
            dx = dh_v[rows, :] + _ln_bwd(daT.T, xhat, rstd)
            dy_v[rows, :] = dx.astype(bf16)
            dx_copy(t).start()

        def tail(t, carry):
            daT = _dot(wqkv_v[...], dQKV[:, t].reshape(3 * D, 128).astype(bf16))
            rows = pl.ds(pl.multiple_of((t % 5) * 128, 128), 128)
            cols = pl.ds(pl.multiple_of(t * 128, 128), 128)
            w = [dflat[t // 5, i, rows, :].astype(bf16) for i in range(NT128)]
            for k in range(4):
                mrows = pl.ds(k * SR, SR)
                last[mrows, :] = (jnp.where(t == 0, 0.0, last[mrows, :])
                                  + _dot(wqkv_v[mrows, cols], w[NT128 - 1]))
            oqkv[:, cols] = _dot_nt(aT[...], jnp.concatenate(w, axis=1)).astype(bf16)
            qkv_copy(t).start()
            dx_finish(t, daT)
            return carry

        with _scope('tail'):
            lax.fori_loop(0, NT128 - 1, tail, 0)
        dx_finish(NT128 - 1, last[...])
        out_copy(NB - 2, 0).wait()
        out_copy(NB - 1, 1).wait()
        for cp in w_copies:
            cp.wait()

        def drain(t, carry):
            qkv_copy(t).wait()
            dx_copy(t).wait()
            return carry

        lax.fori_loop(0, NT128 - 1, drain, 0)
        dx_copy(NT128 - 1).wait()

    pl.run_scoped(epilogue, pltpu.VMEM((D, 3 * D), bf16), pltpu.VMEM((D, 128), f32))


@jax.jit
def pallas_sequential_preLN__softmax_full_mha__glu_gated_geglu__prompt_kernel(
    A_x: jax.Array,
    A_wqkv: jax.Array,
    A_wo: jax.Array,
    B_x: jax.Array,
    B_w_gate: jax.Array,
    B_w_up: jax.Array,
    B_w_down: jax.Array,
    grad_out: jax.Array,
):
    del B_x
    x = A_x.reshape(S, D)
    dy = grad_out.reshape(S, D)
    any_spec = pl.BlockSpec(memory_space=pl.ANY)
    out_shape = (
        jax.ShapeDtypeStruct((S, D), bf16),
        jax.ShapeDtypeStruct((S, D), bf16),
        jax.ShapeDtypeStruct((D, 3 * D), bf16),
        jax.ShapeDtypeStruct((D, D), bf16),
        jax.ShapeDtypeStruct((D, DF), bf16),
        jax.ShapeDtypeStruct((D, DF), bf16),
        jax.ShapeDtypeStruct((DF, D), bf16),
    )
    scratch = [
        pltpu.VMEM((S, D), bf16),
        pltpu.VMEM((S, D), bf16),
        pltpu.VMEM((D, 3 * D), bf16),
        pltpu.VMEM((D, D), bf16),
        pltpu.VMEM((D, DF), bf16),
        pltpu.VMEM((D, DF), bf16),
        pltpu.VMEM((DF, D), bf16),
        pltpu.VMEM((D, S), bf16),
        pltpu.VMEM((NS, BIG_ROWS, 128), u32),
        pltpu.VMEM((NT128, NS, HS, 16, 128), u32),
        pltpu.VMEM((3, NT128, NS, SR, 128), f32),
        pltpu.VMEM((S, D), f32),
        pltpu.VMEM((D, D), f32),
        pltpu.VMEM((D, DF), f32),
        pltpu.VMEM((D, DF), f32),
        pltpu.VMEM((DF, D), f32),
        pltpu.VMEM((NT128, NS, HS, 128), f32),
        pltpu.VMEM((NS, HS, 128), f32),
        pltpu.VMEM((2, TQ, D), bf16),
        pltpu.VMEM((D, DF), bf16),
        pltpu.VMEM((D, DF), bf16),
        pltpu.VMEM((DF, D), bf16),
        pltpu.VMEM((D, D), bf16),
        pltpu.SemaphoreType.DMA((NB,)),
        pltpu.SemaphoreType.DMA((D // WCH,)),
        pltpu.SemaphoreType.DMA((5,)),
        pltpu.SemaphoreType.DMA((2,)),
        pltpu.SemaphoreType.DMA((4,)),
        pltpu.SemaphoreType.DMA((3 * D // 128,)),
        pltpu.SemaphoreType.DMA((NT128,)),
    ]
    out, dx, dwqkv, dwo, dwg, dwu, dwd = pl.pallas_call(
        _kernel,
        out_shape=out_shape,
        in_specs=[any_spec] * 7,
        out_specs=tuple([any_spec] * 7),
        scratch_shapes=scratch,
        compiler_params=pltpu.CompilerParams(vmem_limit_bytes=127 * 1024 * 1024),
    )(x, A_wqkv, A_wo, B_w_gate, B_w_up, B_w_down, dy)
    return (out.reshape(1, S, D), dx.reshape(1, S, D), dwqkv, dwo, dwg, dwu, dwd)
```
